```python
import os as _os
_os.environ.setdefault("JAX_PLATFORMS", "cpu")
import jax
import jax.numpy as jnp

def _softmax(x, axis=-1):
    return jax.nn.softmax(x, axis=axis)
def _gelu(x):
    return jax.nn.gelu(x, approximate=True)
def _silu(x):
    return jax.nn.silu(x)
def _sigmoid(x):
    return jax.nn.sigmoid(x)
def _layernorm(x, axis=-1, eps=1e-5):
    m = jnp.mean(x, axis=axis, keepdims=True)
    v = jnp.var(x, axis=axis, keepdims=True)
    return (x - m) / jnp.sqrt(v + eps)
def _scatter_add(tgt, idx, src, axis=0):
    return tgt.at[idx].add(src)
def _segment_sum(src, seg, n):
    return jax.ops.segment_sum(src, seg, n)
class _Rng:
    def __init__(self, key):
        self._k = key
    def _next(self):
        self._k, sub = jax.random.split(self._k)
        return sub
    def normal(self, shape):
        return jax.random.normal(self._next(), shape, dtype=jnp.bfloat16)
    def randint(self, lo, hi, shape):
        return jax.random.randint(self._next(), shape, lo, hi, dtype=jnp.int32)
    def uniform(self, shape, lo=0.0, hi=1.0):
        return jax.random.uniform(self._next(), shape, jnp.bfloat16, lo, hi)
    def permutation(self, n):
        return jax.random.permutation(self._next(), n)


kernel_name = 'standalone__batchnorm__sampling'

def setup_inputs():
    _rng = _Rng(jax.random.key(int.from_bytes(__import__("os").urandom(4), "little")))
    _w = (lambda a: (lambda t: t.astype(jnp.bfloat16) if jnp.issubdtype(t.dtype, jnp.floating) else t)(jnp.asarray(a)))
    B, S, C = 1024, 8, 640
    K = 3
    return {
        "x": _w((lambda *s: _rng.normal(s) * 0.05)(B, S, C)),
        "w": _w((lambda *s: _rng.normal(s) * 0.05)(K, C, C) * (1.0 / (K * C) ** 0.5)),
        "mean": _w((lambda *s: _rng.normal(s) * 0.05)(C) * 0.1),
        "var": _w(jnp.abs((lambda *s: _rng.normal(s) * 0.05)(C)) + 0.5),
        "g": _w((lambda *s: _rng.normal(s) * 0.05)(C) + 1.0),
        "b": _w((lambda *s: _rng.normal(s) * 0.05)(C) * 0.1),
    }

def reference(x, w, mean, var, g, b):
    K = 3
    P = K // 2
    S = x.shape[1]
    xp = jnp.pad(x, ((0, 0), (P, P), (0, 0)))
    y = sum(jnp.einsum('bsc,cd->bsd', xp[:, k:k + S, :], w[k]) for k in range(K))
    inv_std = 1.0 / jnp.sqrt(var + 1e-5)
    y = (y - mean) * (g * inv_std) + b
    return _silu(y)
```

```python
import functools
import jax, jax.numpy as jnp
from jax import lax
import jax.experimental.pallas as pl
import jax.experimental.pallas.tpu as pltpu

A = 0.625
A2 = A * A
Bp = 1.0 / A
B2 = Bp * Bp
KAP = A2 + B2
NA = 2 * A2 * (A2 - B2)
NB = 2 * B2 * (B2 - A2)
SB = Bp ** 3 / NB
F32 = jnp.float32
BF16 = jnp.bfloat16
U32 = jnp.uint32
NT = 5
C = 640
HI = 0xFFFF0000
TB = 64
B = 1024
NCH = B // TB
H = TB // 2
RB = TB * 8
G = 16
NG = TB // G

def _unpack(v, dep=None):
    if dep is None:
        return (pltpu.bitcast(v << 16, F32), pltpu.bitcast(v & jnp.uint32(HI), F32))
    sh, mask = dep
    return (pltpu.bitcast(v << sh, F32), pltpu.bitcast(v & mask, F32))

def _pack(lo, hi):
    w = pltpu.pack_elementwise([lo, hi], packed_dtype=BF16)
    return w if w.dtype == U32 else pltpu.bitcast(w, U32)

def _mo(i, m):
    return i if isinstance(i, int) else pl.multiple_of(i, m)

def make(margin=2, w0=18, scopes=False, nosemchk=False, nobounds=False, groups=((0, 1, 2), (5, 3, 4)), merge4=True,
         L=2, e_end=16, zin=True, ma=1.5):
    class _Null:
        def __enter__(self): return None
        def __exit__(self, *a): return False
    def scope(name):
        return _Null()
    NIT = (NCH - 4) // L
    assert NIT * L == NCH - 4
    NM = L + 1
    def kern(x_hbm, xt_hbm, w_hbm, mean_hbm, var_hbm, g_hbm, b_hbm, o_hbm,
             xbuf, xtbuf, obuf, wbuf, u_ref, bn0, bn1, bn2, bn3, p_ref, z0_ref, z_ref, vp_ref, v_ref, m_ref, isem, osem):
        xu = xbuf.bitcast(U32)
        ou = obuf.bitcast(U32)
        xtu = xtbuf.bitcast(U32)

        def xk_copy(k, s):
            return pltpu.make_async_copy(x_hbm.at[pl.ds(0, 2 * RB), pl.ds(_mo(k * 128, 128), 128)], xbuf.at[k], isem.at[s])
        def wk_copy(q, k, s):
            r0 = _mo(k * 128, 128)
            return pltpu.make_async_copy(w_hbm.at[q, pl.ds(r0, 128)], wbuf.at[q, pl.ds(r0, 128)], isem.at[s])
        def xt_copy(c0, nc, s):
            return pltpu.make_async_copy(xt_hbm.at[pl.ds(c0 * TB * 40, nc * TB * 40)], xtbuf.at[pl.ds(c0 * TB * 40, nc * TB * 40)], isem.at[s])
        def ok_copy(c, k):
            r0 = _mo(c * RB, RB)
            return pltpu.make_async_copy(obuf.at[k, pl.ds(r0, RB)], o_hbm.at[pl.ds(r0, RB), pl.ds(k * 128, 128)], osem)
        def grp0(): return [xk_copy(0, 0), wk_copy(2, 0, 0)]
        def grp1(): return [wk_copy(0, 0, 1), wk_copy(1, 0, 1), pltpu.make_async_copy(z0_ref, z_ref, isem.at[1])]
        def slab(k): return [xk_copy(k, k + 1)] + [wk_copy(q, k, k + 1) for q in (2, 0, 1)]
        def grp6(): return [xt_copy(2, 2, 6)] + [pltpu.make_async_copy(s_, d, isem.at[6]) for s_, d in zip((mean_hbm, var_hbm, g_hbm, b_hbm), (bn0, bn1, bn2, bn3))]
        n7 = 2 * L if L == 2 else L
        def grp7(): return [xt_copy(4, n7, 7)]
        def grp8(): return [xt_copy(4 + n7, NCH - 4 - n7, 8)]

        def zero_from(m, i=0):
            return pltpu.bitcast(m[8 * i:8 * i + 8, 0:128], U32) & z_ref[...]

        def unit_a(cx, k, t, g, ps, pro, z=None):
            dep = None if z is None else (z | jnp.uint32(16), z | jnp.uint32(HI))
            if pro:
                xg = xu.at[k, pl.ds((cx * TB + g * G) * 4, G * 4)]
                off, bs = 2 * t, 4
            else:
                xg = xtu.at[pl.ds(_mo((cx * TB + g * G) * 20, G * 20), G * 20)]
                off, bs = k * 4 + 2 * t, 20
            vals = []
            for hf in range(2):
                v = {}
                need01 = any(p in ps for p in (0, 1, 3)); need23 = any(p in ps for p in (5, 1, 3))
                if need01: x0, x1 = _unpack(xg[pl.ds(hf * 8 * bs + off, 8, stride=bs), :], dep); v[0] = x0
                if need23: x2, x3 = _unpack(xg[pl.ds(hf * 8 * bs + off + 1, 8, stride=bs), :], dep); v[5] = x3
                if 1 in ps:
                    ea = x0 + A2 * x2; oa = A * (x1 + A2 * x3)
                    v[1] = ea + oa; v[2] = ea - oa
                if 3 in ps:
                    eb = A * (A2 * x0 + x2); ob = A2 * x1 + x3
                    v[3] = eb + ob; v[4] = eb - ob
                vals.append(v)
            rs = pl.ds(t * H + g * 8, 8)
            for p in ps:
                if pro: vp_ref[cx, p, rs, :] = _pack(vals[0][p], vals[1][p])
                else: v_ref[p, k, rs, :] = _pack(vals[0][p], vals[1][p])

        def wraw(q, k, n):
            return pltpu.bitcast(wbuf[q, pl.ds(_mo(k * 128, 128), 128), n * 128:(n + 1) * 128], U32)
        def stage_u(k, n, ps):
            us = pl.ds(_mo(k * 64, 64), 64)
            if 0 in ps: u_ref[0, n, us] = wraw(2, k, n)
            if 5 in ps: u_ref[5, n, us] = wraw(0, k, n)
            if 1 in ps or 3 in ps:
                w0_ = _unpack(wraw(0, k, n)); w1 = _unpack(wraw(1, k, n)); w2 = _unpack(wraw(2, k, n))
                res = {1: [], 2: [], 3: [], 4: []}
                for h in range(2):
                    if 1 in ps:
                        ea = (w2[h] + A2 * w0_[h]) * (1.0 / NA); oa = w1[h] * (A / NA)
                        res[1].append(ea + oa); res[2].append(ea - oa)
                    if 3 in ps:
                        eb = (w2[h] + B2 * w0_[h]) * SB; ob = w1[h] * (Bp * SB)
                        res[3].append(eb + ob); res[4].append(eb - ob)
                for p in ps:
                    if p in res: u_ref[p, n, us] = _pack(res[p][0], res[p][1])

        def unit_c(c, slot, n, g, z=None):
            ns = slice(n * 128, (n + 1) * 128)
            sc = p_ref[0, :, ns]; sh = p_ref[1, :, ns]
            r0 = (g // 2) * 16 + (g % 2)
            Mt = [[m_ref[slot, p, n, pl.ds(t * TB + r0, 8, stride=2), :] for p in range(6)] for t in range(2)]
            def dep(a): return pltpu.bitcast(pltpu.bitcast(a, U32) | z, F32)
            if z is not None and not zin: sc = dep(sc)
            ys = []
            for t in range(2):
                m0, mpa, mma, mpb, mmb, m5 = Mt[t]
                if z is not None and zin:
                    mpa = dep(mpa); mpb = dep(mpb)
                Sa = mpa + mma; Da = mpa - mma; Sb = mpb + mmb; Db = mpb - mmb
                P = Sa + m0
                c4 = P + Sb
                c2 = (-B2) * P - A2 * (Sb + m0)
                c3 = A * Da + Bp * Db - KAP * m5
                c1 = m5 - Bp * Da - A * Db
                if t == 0:
                    c4 = c4 + Mt[1][0]
                else:
                    c1 = c1 + Mt[0][5]
                ys += [c1, c2, c3, c4]
            outs = []
            for y in ys:
                h = y * sc + sh
                outs.append(h * jnp.tanh(h) + h)
            oc = ou.at[n, pl.ds(_mo(c * TB * 4, TB * 4), TB * 4)]
            for j in range(4):
                oc[pl.ds(g * 32 + j, 8, stride=4), :] = _pack(outs[2 * j], outs[2 * j + 1])
            if g == TB // 8 - 1:
                ok_copy(c, n).start()
        def c_units(c, slot):
            return [functools.partial(unit_c, c, slot, n, g) for n in range(NT) for g in range(TB // 8)]

        def run_paced(dots, sched):
            sched = sorted(sched, key=lambda t: t[0])
            si = 0
            for d, dt in enumerate(dots):
                m = dt()
                nrow = m.shape[0] // 8
                zc = {}
                while si < len(sched) and sched[si][0] < d + 1:
                    if len(sched[si]) > 2:
                        sched[si][1](); si += 1; continue
                    i = int((sched[si][0] - d) * nrow)
                    if i not in zc: zc[i] = zero_from(m, i)
                    sched[si][1](z=zc[i]); si += 1
            assert si == len(sched)
        def spread(units, lo, hi):
            n = len(units)
            return [(lo + (hi - lo) * i / n, u) for i, u in enumerate(units)]

        def chunk_dots(c, slot):
            def mk(p, n):
                def f():
                    lhs = jnp.concatenate([pltpu.bitcast(v_ref[p, k], BF16) for k in range(NT)], axis=1)
                    m = jnp.dot(lhs, pltpu.bitcast(u_ref[p, n], BF16), preferred_element_type=F32)
                    m_ref[slot, p, n] = m
                    return m
                return f
            return [mk(p, n) for ps in groups for n in range(NT) for p in ps]
        def a_units(c, gi):
            return [functools.partial(unit_a, c, k, t, g, groups[gi], False) for k in range(NT) for t in range(2) for g in range(NG)]
        def awin(c, base, nxt=True, end=False):
            sch = spread(a_units(c, 1), base + 0.0, base + 15 - ma)
            if nxt: sch += spread(a_units(c + 1, 0), base + 14.5, base + 30 - (margin if end else ma))
            return sch

        pslot = (L, L - 2)
        def p_dots(k, pgroups, first):
            def mk(p, n, pre):
                def f():
                    if pre is not None:
                        for c in range(2):
                            for t in range(2):
                                for g in range(NG): unit_a(c, k, t, g, pre, True)
                        for nn in range(NT): stage_u(k, nn, pre)
                    lhs = jnp.concatenate([pltpu.bitcast(vp_ref[c, p], BF16) for c in range(2)], axis=0)
                    rhs = pltpu.bitcast(u_ref[p, n, pl.ds(_mo(k * 64, 64), 64)], BF16)
                    m = jnp.dot(lhs, rhs, preferred_element_type=F32)
                    for c in range(2):
                        piece = m[c * 128:(c + 1) * 128]
                        if first: m_ref[pslot[c], p, n] = piece
                        else: m_ref[pslot[c], p, n] += piece
                    return m
                return f
            return [mk(p, n, ps if (n == 0 and p == ps[0]) else None) for ps in pgroups for n in range(NT) for p in ps]
        PG = ((0,), (5,), (1, 2), (3, 4))

        z0_ref[...] = jnp.zeros((8, 128), U32)
        for grp in (grp0(), grp1(), slab(1), slab(2), slab(3), slab(4), grp6(), grp7(), grp8()):
            for cp in grp: cp.start()

        with scope("waitP0a"):
            for cp in grp0(): cp.wait()
        run_paced(p_dots(0, PG[:1], True), [])
        with scope("waitP0b"):
            for cp in grp1(): cp.wait()
        run_paced(p_dots(0, PG[1:], True), [])
        def pbody(k, carry):
            with scope("waitP"):
                for cp in slab(k): cp.wait()
            run_paced(p_dots(k, PG, False), [])
            return carry
        lax.fori_loop(1, NT - 1 if merge4 else NT, pbody, 0)

        with scope("waitR0"):
            if merge4:
                for cp in slab(4): cp.wait()
            for cp in grp6(): cp.wait()
        mean, var, g, b = [q[...].astype(F32).reshape(1, C) for q in (bn0, bn1, bn2, bn3)]
        sc = g / jnp.sqrt(var + 1e-5)
        p_ref[0] = jnp.broadcast_to(0.5 * sc, (8, C))
        p_ref[1] = jnp.broadcast_to(0.5 * (b - mean * sc), (8, C))
        assert merge4
        run_paced(p_dots(4, PG, False), spread(a_units(2, 0), 3, 27))
        nhead = int(round(40 * (30 - margin - w0) / 30))
        def cwin(c, slot, base, lo_unit=0, hi_unit=40, shift=0.0):
            us = c_units(c, slot)
            return [(base + w0 + 30.0 * i / 40 + shift, us[i]) for i in range(lo_unit, hi_unit)]
        sched = spread(c_units(0, pslot[0]) + c_units(1, pslot[1]), 0.5, 30 - margin - 0.01) + cwin(2, L - 1, 0, 0, nhead) + awin(2, 0, end=True)
        run_paced(chunk_dots(2, L - 1), sched)

        def body(it, carry):
            c = L * it + 3
            with scope("waitL"):
                @pl.when(it == 0)
                def _():
                    for cp in grp7(): cp.wait()
                @pl.when(it == n7 // L)
                def _():
                    for cp in grp8(): cp.wait()
            dots = [d for j in range(L) for d in chunk_dots(c + j, j)]
            sched = cwin(c - 1, L - 1, -30, nhead, 40, shift=margin + 0.5)
            for j in range(L):
                sched += cwin(c + j, j, 30 * j, 0, 40 if j < L - 1 else nhead) + awin(c + j, 30 * j, end=(j == L - 1))
            run_paced(dots, sched)
            return carry
        lax.fori_loop(0, NIT, body, 0)

        cl = NCH - 1
        us = c_units(cl - 1, L - 1)[nhead:]
        sched = spread(us, 0.5, e_end) + awin(cl, 0, nxt=False)
        ng = len(groups[-1]); base = 30 - NT * ng
        ul = c_units(cl, 0)
        for n in range(NT):
            for g in range(8):
                sched.append((base + (n + 1) * ng - 0.5, ul[n * 8 + g], True))
        run_paced(chunk_dots(cl, 0), sched)
        with scope("waitEnd"):
            for c in range(NCH):
                for k in range(NT): ok_copy(c, k).wait()

    def f(x, w, mean, var, g, b):
        Bx, S, Cx = x.shape
        xt = x.reshape(B * S, Cx)
        xtile = x.reshape(B, S, NT, 128).transpose(0, 2, 1, 3).reshape(B * 40, 128)
        anyspec = pl.BlockSpec(memory_space=pl.ANY)
        out = pl.pallas_call(
            kern,
            in_specs=[anyspec] * 7,
            out_specs=anyspec,
            out_shape=jax.ShapeDtypeStruct(xt.shape, x.dtype),
            scratch_shapes=[
                pltpu.VMEM((NT, 2 * RB, 128), BF16), pltpu.VMEM((B * 40, 128), BF16), pltpu.VMEM((NT, B * 8, 128), BF16),
                pltpu.VMEM((3, C, C), BF16), pltpu.VMEM((6, NT, C // 2, 128), U32),
                pltpu.VMEM((C,), BF16), pltpu.VMEM((C,), BF16), pltpu.VMEM((C,), BF16), pltpu.VMEM((C,), BF16),
                pltpu.VMEM((2, 8, C), F32), pltpu.VMEM((8, 128), U32), pltpu.VMEM((8, 128), U32),
                pltpu.VMEM((2, 6, TB, 128), U32), pltpu.VMEM((6, NT, TB, 128), U32),
                pltpu.VMEM((NM, 6, NT, 2 * TB, 128), F32),
                pltpu.SemaphoreType.DMA((9,)), pltpu.SemaphoreType.DMA,
            ],
            compiler_params=pltpu.CompilerParams(vmem_limit_bytes=64 * 1024 * 1024,
                                                 disable_semaphore_checks=nosemchk, disable_bounds_checks=nobounds),
        )(xt, xtile, w, mean, var, g, b)
        return out.reshape(B, S, Cx)
    return f


_impl = make(nobounds=True, nosemchk=True, zin=False, w0=26)


@jax.jit
def pallas_standalone__batchnorm__sampling_kernel(x, w, mean, var, g, b):
    return _impl(x, w, mean, var, g, b)
```

```python
import functools
import jax, jax.numpy as jnp
from jax import lax
import jax.experimental.pallas as pl
import jax.experimental.pallas.tpu as pltpu

A = 0.5
AL = A * A
Bp = 1.0 / A
_A1 = 1 + AL ** 3; _A2 = AL + AL ** 2; _B1 = 1 - AL ** 3; _B2 = AL - AL ** 2
_KAP = _A1 - _A2
MUA = 1 / (2 * AL * _KAP); MUB = MUA * A
K1 = _A1 / _KAP
K3 = (1 / AL + AL ** 4) / _KAP - K1
K4 = _KAP / (_B1 + _B2); K6 = _B1 / (_B1 + _B2)
F32 = jnp.float32
BF16 = jnp.bfloat16
U32 = jnp.uint32
NT = 5
C = 640
HI = 0xFFFF0000
TB = 128
B = 1024
NCH = B // TB
RB = TB * 8
G = 16
NG = TB // G
NP = 11
G0 = (0, 1, 2, 3, 4, 5)
G1 = (6, 7, 8, 9, 10)

def _bits(a): return pltpu.bitcast(a, U32)

def _unpack(v, dep=None):
    if dep is None:
        return (pltpu.bitcast(v << 16, F32), pltpu.bitcast(v & jnp.uint32(HI), F32))
    sh, mask = dep
    return (pltpu.bitcast(v << sh, F32), pltpu.bitcast(v & mask, F32))

def _pack(lo, hi, mode):
    if mode == "elem":
        w = pltpu.pack_elementwise([lo, hi], packed_dtype=BF16)
        return w if w.dtype == U32 else pltpu.bitcast(w, U32)
    if mode == "rne":
        return (_bits(lo.astype(BF16).astype(F32)) >> 16) | _bits(hi.astype(BF16).astype(F32))
    if mode == "exact":
        return (_bits(lo) >> 16) | _bits(hi)
    assert mode == "int"
    return ((_bits(lo) + jnp.uint32(0x8000)) >> 16) | ((_bits(hi) + jnp.uint32(0x8000)) & jnp.uint32(HI))

def _mo(i, m):
    return i if isinstance(i, int) else pl.multiple_of(i, m)

def make(scopes=False, nosemchk=True, nobounds=True, L=2, n0a=1, pv='int', pu='int', po='rne',
         ma=1.0, margin=2.5, a_lo=0.2, c_lo=5.5, c_hi=52.0, zin=True, asub=False, esplit=2, pm=5.0, plo=0.3, unat=True, pg0a=None,
         pg=((0,), (1,), (2, 3, 6, 7, 8), (4, 5), (9, 10)), r0a=(0.2, 4.0, 9.0, 18.5, 12.0), mr0=1.5):
    class _Null:
        def __enter__(self): return None
        def __exit__(self, *a): return False
    def scope(name):
        return _Null()
    NSEG = NCH - 2
    NIT = NSEG // L
    assert NIT * L == NSEG
    XB = 96 // NIT
    assert XB % 16 == 0
    def kern(x_hbm, xt_hbm, w_hbm, mean_hbm, var_hbm, g_hbm, b_hbm, o_hbm,
             xbuf, xtbuf, obuf, obuf0, wbuf, u_ref, bn0, bn1, bn2, bn3, p_ref, z0_ref, z_ref, vp_ref, v_ref, mp_ref, m_ref, isem, osem):
        xu = xbuf.bitcast(U32)
        ou = obuf.bitcast(U32)
        ou0 = obuf0.bitcast(U32)
        xtu = xtbuf.bitcast(U32)
        uu = u_ref.bitcast(U32) if unat else u_ref

        def xk_copy(k, s):
            return pltpu.make_async_copy(x_hbm.at[pl.ds(0, 2 * RB), pl.ds(_mo(k * 128, 128), 128)], xbuf.at[k], isem.at[s])
        def xk0_copy(c, s):
            return pltpu.make_async_copy(x_hbm.at[pl.ds(c * RB, RB), pl.ds(0, 128)], xbuf.at[0, pl.ds(c * RB, RB)], isem.at[s])
        def wk_copy(q, k, s):
            r0 = _mo(k * 128, 128)
            return pltpu.make_async_copy(w_hbm.at[q, pl.ds(r0, 128)], wbuf.at[q, pl.ds(r0, 128)], isem.at[s])
        def wkn_copy(q, n0_, n1_, s):
            cs = pl.ds(n0_ * 128, (n1_ - n0_) * 128)
            return pltpu.make_async_copy(w_hbm.at[q, pl.ds(0, 128), cs], wbuf.at[q, pl.ds(0, 128), cs], isem.at[s])
        def xt_copy(c0, nc, s):
            return pltpu.make_async_copy(xt_hbm.at[pl.ds(c0 * TB * 40, nc * TB * 40)], xtbuf.at[pl.ds(c0 * TB * 40, nc * TB * 40)], isem.at[s])
        def o_copy(b0, nb, k, first):
            r0 = _mo(b0 * 8, 128)
            src = obuf0 if first else obuf
            return pltpu.make_async_copy(src.at[k, pl.ds(r0, nb * 8)], o_hbm.at[pl.ds(r0, nb * 8), pl.ds(k * 128, 128)], osem)
        bn_copies = lambda s: [pltpu.make_async_copy(s_, d, isem.at[s]) for s_, d in zip((mean_hbm, var_hbm, g_hbm, b_hbm), (bn0, bn1, bn2, bn3))]
        def grp0(): return [xk0_copy(0, 0)] + [wkn_copy(q, 0, n0a, 0) for q in (2, 0, 1)] + [pltpu.make_async_copy(z0_ref, z_ref, isem.at[0])]
        def grp1(): return [wkn_copy(q, n0a, NT, 1) for q in (2, 0, 1)] + [xk0_copy(1, 1)] + bn_copies(1)
        def slab(k): return [xk_copy(k, k + 1)] + [wk_copy(q, k, k + 1) for q in (2, 0, 1)]
        def grp7(): return [xt_copy(2, L, 6)]
        def grp8(): return [xt_copy(2 + L, NCH - 2 - L, 7)]

        def zero_from(m, i=0):
            return _bits(m[8 * i:8 * i + 8, 0:128]) & z_ref[...]

        def unit_a(cx, k, g, ps, pro, z=None):
            dep = None if z is None else (z | jnp.uint32(16), z | jnp.uint32(HI))
            if pro:
                xg = xu.at[k, pl.ds((cx * TB + g * G) * 4, G * 4)]
                off, bs = 0, 4
            else:
                xg = xtu.at[pl.ds(_mo((cx * TB + g * G) * 20, G * 20), G * 20)]
                off, bs = k * 4, 20
            full = any(p >= 2 for p in ps)
            vals = []
            for hf in range(2):
                x = {}
                for j in range(4):
                    if full or (j == 0 and 0 in ps) or (j == 3 and 1 in ps):
                        x[2 * j], x[2 * j + 1] = _unpack(xg[pl.ds(hf * 8 * bs + off + j, 8, stride=bs), :], dep)
                v = {}
                if 0 in ps: v[0] = x[0]
                if 1 in ps: v[1] = x[7]
                if 2 in ps or 6 in ps:
                    p_ = x[0] + x[4]; q_ = x[2] + x[6]; r_ = x[1] + x[5]; s_ = x[3] + x[7]
                if 2 in ps:
                    e1 = p_ + q_; o1 = r_ + s_
                    v[2] = e1 + o1; v[3] = e1 - o1
                if 6 in ps:
                    ei = p_ - q_; oi = r_ - s_
                    v[6] = ei + oi; v[7] = ei; v[8] = oi
                if 4 in ps:
                    ea = x[0] + AL * (x[2] + AL * (x[4] + AL * x[6])); oa = A * (x[1] + AL * (x[3] + AL * (x[5] + AL * x[7])))
                    v[4] = ea + oa; v[5] = ea - oa
                if 9 in ps:
                    eb = A * (x[6] + AL * (x[4] + AL * (x[2] + AL * x[0]))); ob = x[7] + AL * (x[5] + AL * (x[3] + AL * x[1]))
                    v[9] = eb + ob; v[10] = eb - ob
                vals.append(v)
            rs = pl.ds(g * 8, 8)
            for p in ps:
                md = "exact" if (p in (0, 1) and pv != "elem") else pv
                if pro and not (cx == 1 and p in G1): vp_ref[p, pl.ds(cx * (TB // 2) + g * 8, 8), :] = _pack(vals[0][p], vals[1][p], md)
                else: v_ref[p, k, rs, :] = _pack(vals[0][p], vals[1][p], md)

        def wraw(q, k, n):
            return _bits(wbuf[q, pl.ds(_mo(k * 128, 128), 128), n * 128:(n + 1) * 128])
        def stage_u_nat(k, n, ps):
            us = pl.ds(_mo(k * 128, 128), 128)
            wr = lambda q: wbuf[q, us, n * 128:(n + 1) * 128]
            if 0 in ps: u_ref[0, n, us] = wr(2)
            if 1 in ps: u_ref[1, n, us] = wr(0)
            if any(p >= 2 for p in ps):
                w0, w1, w2 = [wr(q).astype(F32) for q in range(3)]
                r = {}
                if 2 in ps:
                    e = 0.5 * (w2 + w0); o = 0.5 * w1
                    r[2] = e + o; r[3] = e - o
                if 6 in ps:
                    gr = w2 - w0
                    r[6] = gr; r[7] = w1 - gr; r[8] = gr + w1
                if 4 in ps:
                    e = MUA * (w2 + AL * w0); o = (MUA * A) * w1
                    r[4] = e + o; r[5] = e - o
                if 9 in ps:
                    e = MUB * (AL * w2 + w0); o = (MUB * A) * w1
                    r[9] = e + o; r[10] = e - o
                for p in ps:
                    if p >= 2: u_ref[p, n, us] = r[p].astype(BF16)
        def stage_u(k, n, ps):
            if unat: return stage_u_nat(k, n, ps)
            us = pl.ds(_mo(k * 64, 64), 64)
            if 0 in ps: u_ref[0, n, us] = wraw(2, k, n)
            if 1 in ps: u_ref[1, n, us] = wraw(0, k, n)
            if any(p >= 2 for p in ps):
                w0_ = _unpack(wraw(0, k, n)); w1_ = _unpack(wraw(1, k, n)); w2_ = _unpack(wraw(2, k, n))
                res = [{}, {}]
                for h in range(2):
                    w0, w1, w2, r = w0_[h], w1_[h], w2_[h], res[h]
                    if 2 in ps:
                        e = 0.5 * (w2 + w0); o = 0.5 * w1
                        r[2] = e + o; r[3] = e - o
                    if 6 in ps:
                        gr = w2 - w0
                        r[6] = gr; r[7] = w1 - gr; r[8] = gr + w1
                    if 4 in ps:
                        e = MUA * (w2 + AL * w0); o = (MUA * A) * w1
                        r[4] = e + o; r[5] = e - o
                    if 9 in ps:
                        e = MUB * (AL * w2 + w0); o = (MUB * A) * w1
                        r[9] = e + o; r[10] = e - o
                for p in ps:
                    if p >= 2: u_ref[p, n, us] = _pack(res[0][p], res[1][p], pu)

        def unit_c(mview, b0, nb, first, n, g, z=None):
            ns = slice(n * 128, (n + 1) * 128)
            sc = p_ref[0, :, ns]; sh = p_ref[1, :, ns]
            dp = lambda a: pltpu.bitcast(_bits(a) | z, F32)
            if z is not None and not zin: sc = dp(sc)
            m0, mi, mp1, mm1, mpa, mma, q1, q2, q3, mpb, mmb = [
                mview(p, n)[pl.ds((g // 2) * 16 + (g % 2), 8, stride=2), :] for p in range(NP)]
            if z is not None and zin: mp1, mpa, mpb, q1 = dp(mp1), dp(mpa), dp(mpb), dp(q1)
            S1 = mp1 + mm1; D1 = mp1 - mm1; Sa = mpa + mma; Da = mpa - mma; Sb = mpb + mmb; Db = mpb - mmb
            Re = q1 - q3; Im = q1 + q2
            km0 = K3 * m0; kmi = K3 * mi
            s2 = (K1 * S1 - (Sa + Sb)) + km0; s1 = (S1 - m0) - s2
            d2 = (K4 * (Sa - Sb) + K6 * Re) - km0; d1 = (m0 - Re) + d2
            aDa = A * Da; bDb = Bp * Db
            t2 = (K1 * D1 - (aDa + bDb)) + kmi; t1 = (D1 - mi) - t2
            e2 = (K4 * (aDa - bDb) - K6 * Im) + kmi; e1 = (Im - mi) + e2
            ys = [t1 + e1, s1 + d1, t2 + e2, s2 + d2, t2 - e2, s2 - d2, t1 - e1, s1 - d1]
            outs = []
            for y in ys:
                h = y * sc + sh
                outs.append(h * jnp.tanh(h) + h)
            oc = (ou0 if first else ou).at[n, pl.ds(_mo(b0 * 4, 64), nb * 4)]
            for j in range(4):
                oc[pl.ds(g * 32 + j, 8, stride=4), :] = _pack(outs[2 * j], outs[2 * j + 1], po)
            if g == nb // 8 - 1:
                o_copy(b0, nb, n, first).start()
        def c_units(c, slot):
            mv = lambda p, n: m_ref.at[slot, p, n]
            return [functools.partial(unit_c, mv, c * TB, TB, False, n, g) for n in range(NT) for g in range(TB // 8)]
        def cx_units(b0, nb):
            mv = lambda p, n: mp_ref.at[p, n, pl.ds(_mo(b0, 16), nb)]
            return [functools.partial(unit_c, mv, b0, nb, True, n, g) for n in range(NT) for g in range(nb // 8)]

        def run_paced(dots, sched):
            sched = sorted(sched, key=lambda t: t[0])
            si = 0
            for d, dt in enumerate(dots):
                m = dt()
                nrow = m.shape[0] // 8
                zc = {}
                while si < len(sched) and sched[si][0] < d + 1:
                    if len(sched[si]) > 2:
                        sched[si][1](); si += 1; continue
                    i = int((sched[si][0] - d) * nrow)
                    if i not in zc: zc[i] = zero_from(m, i)
                    sched[si][1](z=zc[i]); si += 1
            assert si == len(sched)
        def spread(units, lo, hi):
            n = len(units)
            return [(lo + (hi - lo) * i / n, u) for i, u in enumerate(units)]

        def mk_dot(slot, p, n):
            def f():
                lhs = jnp.concatenate([pltpu.bitcast(v_ref[p, k], BF16) for k in range(NT)], axis=1)
                m = jnp.dot(lhs, pltpu.bitcast(uu[p, n], BF16), preferred_element_type=F32)
                m_ref[slot, p, n] = m
                return m
            return f
        def gdots(ps, slot): return [mk_dot(slot, p, n) for n in range(NT) for p in ps]
        def a_units(c, ps):
            subs = {G0: ((0, 1, 2, 3), (4, 5)), G1: ((6, 7, 8), (9, 10))}.get(ps, (ps,)) if asub else (ps,)
            return [functools.partial(unit_a, c, k, g, sb, False) for g in range(NG) for k in range(NT) for sb in subs]

        def p_step(k, first, jobs, a_chunks, u_ns, pace=True, pg=pg):
            def mk(p, n, cs, pre):
                def f():
                    for fn in pre: fn()
                    h = TB // 2
                    lhs = pltpu.bitcast(vp_ref[p, cs[0] * h:(cs[-1] + 1) * h], BF16)
                    rhs = pltpu.bitcast(uu[p, n, pl.ds(_mo(k * 64, 64), 64)], BF16)
                    m = jnp.dot(lhs, rhs, preferred_element_type=F32)
                    for i, cx in enumerate(cs):
                        dst = mp_ref.at[p, n] if cx == 0 else m_ref.at[0, p, n]
                        piece = m[i * TB:(i + 1) * TB]
                        if first: dst[...] = piece
                        else: dst[...] += piece
                    return m
                return f
            dots, sched = [], []
            lo = plo
            for gi, ps in enumerate(pg):
                lst = sorted([(n, ps.index(p), p, cs) for p in ps for (n, cs) in jobs(p)])
                aus = [functools.partial(unit_a, cx, k, g, ps, True) for cx in a_chunks for g in range(NG)]
                start = len(dots)
                pre = [functools.partial(stage_u, k, nn, ps) for nn in u_ns]
                if pace and len(ps) > 1 and start - pm > lo:
                    sched += spread(aus, lo, start - pm)
                    lo = start - pm
                else:
                    pre = aus + pre
                for i, (n, _, p, cs) in enumerate(lst):
                    dots.append(mk(p, n, cs, pre if i == 0 else []))
            run_paced(dots, sched)
        both = lambda p: (0, 1) if p in G0 else (0,)

        z0_ref[...] = jnp.zeros((8, 128), U32)
        for grp in (grp0(), grp1(), slab(1), slab(2), slab(3), slab(4), grp7(), grp8()):
            for cp in grp: cp.start()

        with scope("waitP0a"):
            for cp in grp0(): cp.wait()
        p_step(0, True, lambda p: [(n, (0,)) for n in range(n0a)], (0,), range(n0a), pace=False, pg=pg0a or pg)
        with scope("waitP0b"):
            for cp in grp1(): cp.wait()
        mean, var, g, b = [q[...].astype(F32).reshape(1, C) for q in (bn0, bn1, bn2, bn3)]
        sc = g / jnp.sqrt(var + 1e-5)
        p_ref[0] = jnp.broadcast_to(0.25 * sc, (8, C))
        p_ref[1] = jnp.broadcast_to(0.5 * (b - mean * sc), (8, C))
        p_step(0, True, lambda p: ([(n, (1,)) for n in range(n0a)] if p in G0 else []) + [(n, both(p)) for n in range(n0a, NT)],
               (1,), range(n0a, NT))
        def pbody(k, carry):
            with scope("waitP"):
                for cp in slab(k): cp.wait()
            p_step(k, False, lambda p: [(n, both(p)) for n in range(NT)], (0, 1), range(NT))
            return carry
        lax.fori_loop(1, NT, pbody, 0)

        def body(it, carry):
            with scope("waitL"):
                @pl.when(it == 0)
                def _():
                    for cp in grp7(): cp.wait()
                @pl.when(it == 1)
                def _():
                    for cp in grp8(): cp.wait()
            dots, sched = [], []
            xun = cx_units(it * XB, XB)
            per = len(xun) // L
            for j in range(L):
                c = L * it + 1 + j
                base = 55 * j
                dots += gdots(G1, j % L) + gdots(G0, (j + 1) % L)
                endm = margin if j == L - 1 else ma
                sched += spread(a_units(c + 1, G0), base + a_lo, base + 25 - ma)
                sched += spread(a_units(c + 1, G1), base + 24.6, base + 55 - endm)
                cs = spread(c_units(c, j % L), base + c_lo, base + c_hi)
                for pos, u in cs:
                    n = u.args[4]
                    assert base + 5 * n + 4 <= pos and (L > 1 or pos < base + 25 + 6 * n), (pos, n)
                sched += cs
                xs = xun[j * per:(j + 1) * per]
                sched += spread(xs, base + 0.4, base + c_lo)
            run_paced(dots, sched)
            return carry
        lax.fori_loop(0, NIT, body, 0)

        cl = NCH - 1
        sched = spread(cx_units(96, 32), 0.3, 5.0)
        ul = c_units(cl, 0)
        for n in range(NT - 1):
            for g in range(16):
                span = 4.9 if n < NT - 2 else 5.0 * esplit - 5.5 if esplit > 1 else 3.5
                sched.append((5 * (n + 1) + span * g / 16, ul[n * 16 + g]))
        nb = TB // esplit
        def mk_part(p, h):
            def f():
                rs = slice(h * nb // 2, (h + 1) * nb // 2)
                lhs = jnp.concatenate([pltpu.bitcast(v_ref[p, k, rs], BF16) for k in range(NT)], axis=1)
                m = jnp.dot(lhs, pltpu.bitcast(uu[p, NT - 1], BF16), preferred_element_type=F32)
                m_ref[0, p, NT - 1, h * nb:(h + 1) * nb] = m
                return m
            return f
        edots = gdots(G1, 0)[:20] + [mk_part(p, h) for h in range(esplit) for p in G1]
        for h in range(esplit):
            mv = lambda p, n, h=h: m_ref.at[0, p, n, pl.ds(h * nb, nb)]
            for g in range(nb // 8):
                sched.append((20 + 5 * (h + 1) - 0.5, functools.partial(unit_c, mv, cl * TB + h * nb, nb, False, NT - 1, g), True))
        with scope("E"):
            run_paced(edots, sched)
        with scope("waitEnd"):
            for k in range(NT):
                for it in range(NIT): o_copy(it * XB, XB, k, True).wait()
                o_copy(96, 32, k, True).wait()
                for c in range(1, NCH):
                    if (c, k) != (cl, NT - 1): o_copy(c * TB, TB, k, False).wait()
            for h in range(esplit): o_copy(cl * TB + h * nb, nb, NT - 1, False).wait()

    def f(x, w, mean, var, g, b):
        Bx, S, Cx = x.shape
        xt = x.reshape(B * S, Cx)
        xtile = x.reshape(B, S, NT, 128).transpose(0, 2, 1, 3).reshape(B * 40, 128)
        anyspec = pl.BlockSpec(memory_space=pl.ANY)
        out = pl.pallas_call(
            kern,
            in_specs=[anyspec] * 7,
            out_specs=anyspec,
            out_shape=jax.ShapeDtypeStruct(xt.shape, x.dtype),
            scratch_shapes=[
                pltpu.VMEM((NT, 2 * RB, 128), BF16), pltpu.VMEM((B * 40, 128), BF16), pltpu.VMEM((NT, B * 8, 128), BF16), pltpu.VMEM((NT, RB, 128), BF16),
                pltpu.VMEM((3, C, C), BF16), pltpu.VMEM((NP, NT, C, 128), BF16) if unat else pltpu.VMEM((NP, NT, C // 2, 128), U32),
                pltpu.VMEM((C,), BF16), pltpu.VMEM((C,), BF16), pltpu.VMEM((C,), BF16), pltpu.VMEM((C,), BF16),
                pltpu.VMEM((2, 8, C), F32), pltpu.VMEM((8, 128), U32), pltpu.VMEM((8, 128), U32),
                pltpu.VMEM((NP, TB, 128), U32), pltpu.VMEM((NP, NT, TB // 2, 128), U32),
                pltpu.VMEM((NP, NT, TB, 128), F32), pltpu.VMEM((L, NP, NT, TB, 128), F32),
                pltpu.SemaphoreType.DMA((8,)), pltpu.SemaphoreType.DMA,
            ],
            compiler_params=pltpu.CompilerParams(vmem_limit_bytes=64 * 1024 * 1024,
                                                 disable_semaphore_checks=nosemchk, disable_bounds_checks=nobounds),
        )(xt, xtile, w, mean, var, g, b)
        return out.reshape(B, S, Cx)
    return f


_impl = make(unat=False, n0a=3, pg0a=((0,), (2, 3, 6, 7, 8), (9, 10, 1), (4, 5)))


@jax.jit
def pallas_standalone__batchnorm__sampling_kernel(x, w, mean, var, g, b):
    return _impl(x, w, mean, var, g, b)
```

```python
import functools

import jax
import jax.numpy as jnp
from jax import lax
import jax.experimental.pallas as pl
import jax.experimental.pallas.tpu as pltpu

F32 = jnp.float32
BF16 = jnp.bfloat16
U32 = jnp.uint32

B = 1024
S = 8
C = 640
NT = C // 128
TB = 128
NCH = B // TB
RB = TB * S
G = 16
NG = TB // G
HI = 0xFFFF0000

NP = 11
G0 = (0, 1, 2, 3, 4, 5)
G1 = (6, 7, 8, 9, 10)
RAW = {0: 2, 1: 0}
A = 0.5
AL = A * A
_A1 = 1 + AL ** 3
_A2 = AL + AL ** 2
_B1 = 1 - AL ** 3
_B2 = AL - AL ** 2
_KAP = _A1 - _A2
MUA = 1 / (2 * AL * _KAP)
MUB = MUA * A
K1 = _A1 / _KAP
K3 = (1 / AL + AL ** 4) / _KAP - K1
K4 = _KAP / (_B1 + _B2)
K6 = _B1 / (_B1 + _B2)

L = 2
NIT = (NCH - 2) // L
XB = 96 // NIT
N0A = 3
ESPLIT = 4
PG = ((0,), (1,), (2, 3, 6, 7, 8), (4, 5), (9, 10))
PG0A = ((0,), (1,), (2, 3, 6, 7, 8), (4, 5, 9, 10))
PM, PLO = 3.6, 0.08
MA, MARGIN, A_LO, A1_LO, C_HI, X_LO, U_LO = 0.43, 1.79, 0.66, 24.9, 54.75, 0.5, 0.09
COST_A, COST_C = 140.0, 110.0
EX, ESPAN, ESPAN3, E_OFF = (0.08, 4.8), 4.6, 18.33, -0.1


def _bits(a):
    return pltpu.bitcast(a, U32)


def _f32(a):
    return pltpu.bitcast(a, F32)


def _unpack(v, dep=None):
    if dep is None:
        return _f32(v << 16), _f32(v & jnp.uint32(HI))
    sh, mask = dep
    return _f32(v << sh), _f32(v & mask)


def _pack_exact(lo, hi):
    return (_bits(lo) >> 16) | _bits(hi)


def _pack_round(lo, hi):
    half = jnp.uint32(0x8000)
    return ((_bits(lo) + half) >> 16) | ((_bits(hi) + half) & jnp.uint32(HI))


def _pack_rne(lo, hi):
    return _pack_exact(lo.astype(BF16).astype(F32), hi.astype(BF16).astype(F32))


def _mo(i, m):
    return i if isinstance(i, int) else pl.multiple_of(i, m)


def _spread(units, lo, hi):
    n = len(units)
    return [(lo + (hi - lo) * i / n, u) for i, u in enumerate(units)]


def _kernel(x_hbm, xt_hbm, w_hbm, mean_hbm, var_hbm, g_hbm, b_hbm, o_hbm,
            xbuf, xtbuf, obuf, obuf0, wbuf, u_ref, bn0, bn1, bn2, bn3, p_ref, z0_ref, z_ref,
            vp_ref, v_ref, mp_ref, m_ref, isem, osem):
    xu = xbuf.bitcast(U32)
    xtu = xtbuf.bitcast(U32)
    ou = obuf.bitcast(U32)
    ou0 = obuf0.bitcast(U32)
    wu = wbuf.bitcast(U32)

    def xk_copy(k, s):
        return pltpu.make_async_copy(
            x_hbm.at[pl.ds(0, 2 * RB), pl.ds(_mo(k * 128, 128), 128)], xbuf.at[k], isem.at[s])

    def xk0_copy(c, s):
        return pltpu.make_async_copy(
            x_hbm.at[pl.ds(c * RB, RB), pl.ds(0, 128)], xbuf.at[0, pl.ds(c * RB, RB)], isem.at[s])

    def wn_copy(k, n, s):
        r0 = _mo(k * 128, 128)
        return pltpu.make_async_copy(
            w_hbm.at[:, pl.ds(r0, 128), pl.ds(n * 128, 128)], wbuf.at[n, :, pl.ds(r0, 128)], isem.at[s])

    def xt_copy(c0, nc, s):
        rows = pl.ds(c0 * TB * 40, nc * TB * 40)
        return pltpu.make_async_copy(xt_hbm.at[rows], xtbuf.at[rows], isem.at[s])

    def o_copy(b0, nb, k, first):
        r0 = _mo(b0 * S, 128)
        src = obuf0 if first else obuf
        return pltpu.make_async_copy(
            src.at[k, pl.ds(r0, nb * S)], o_hbm.at[pl.ds(r0, nb * S), pl.ds(k * 128, 128)], osem)

    def grp_x():
        return [xk0_copy(0, 8)]

    def grp_0a():
        return [wn_copy(0, n, 0) for n in range(N0A)] + [pltpu.make_async_copy(z0_ref, z_ref, isem.at[0])]

    def grp_0b():
        return ([wn_copy(0, n, 1) for n in range(N0A, NT)] + [xk0_copy(1, 1)]
                + [pltpu.make_async_copy(s_, d_, isem.at[1])
                   for s_, d_ in zip((mean_hbm, var_hbm, g_hbm, b_hbm), (bn0, bn1, bn2, bn3))])

    def slab(k):
        return [xk_copy(k, k + 1)] + [wn_copy(k, n, k + 1) for n in range(NT)]

    def grp_l0():
        return [xt_copy(2, L, 6)]

    def grp_l1():
        return [xt_copy(2 + L, NCH - 2 - L, 7)]

    def zero_from(m, i):
        return _bits(m[8 * i:8 * i + 8, 0:128]) & z_ref[...]

    def unit_a(cx, k, g, ps, pro, z=None):
        dep = None if z is None else (z | jnp.uint32(16), z | jnp.uint32(HI))
        if pro:
            xg = xu.at[k, pl.ds((cx * TB + g * G) * 4, G * 4)]
            off, bs = 0, 4
        else:
            xg = xtu.at[pl.ds(_mo((cx * TB + g * G) * 20, G * 20), G * 20)]
            off, bs = k * 4, 20
        full = any(p >= 2 for p in ps)
        vals = []
        for hf in range(2):
            x = {}
            for j in range(4):
                if full or (j == 0 and 0 in ps) or (j == 3 and 1 in ps):
                    x[2 * j], x[2 * j + 1] = _unpack(xg[pl.ds(hf * 8 * bs + off + j, 8, stride=bs), :], dep)
            v = {}
            if 0 in ps:
                v[0] = x[0]
            if 1 in ps:
                v[1] = x[7]
            if 2 in ps or 6 in ps:
                p_ = x[0] + x[4]
                q_ = x[2] + x[6]
                r_ = x[1] + x[5]
                s_ = x[3] + x[7]
            if 2 in ps:
                e1 = p_ + q_
                o1 = r_ + s_
                v[2] = e1 + o1
                v[3] = e1 - o1
            if 6 in ps:
                ei = p_ - q_
                oi = r_ - s_
                v[6] = ei + oi
                v[7] = ei
                v[8] = oi
            if 4 in ps:
                ea = x[0] + AL * (x[2] + AL * (x[4] + AL * x[6]))
                oa = A * (x[1] + AL * (x[3] + AL * (x[5] + AL * x[7])))
                v[4] = ea + oa
                v[5] = ea - oa
            if 9 in ps:
                eb = A * (x[6] + AL * (x[4] + AL * (x[2] + AL * x[0])))
                ob = x[7] + AL * (x[5] + AL * (x[3] + AL * x[1]))
                v[9] = eb + ob
                v[10] = eb - ob
            vals.append(v)
        for p in ps:
            w = (_pack_exact if p in RAW else _pack_round)(vals[0][p], vals[1][p])
            if pro and not (cx == 1 and p in G1):
                vp_ref[p, pl.ds(cx * (TB // 2) + g * 8, 8), :] = w
            else:
                v_ref[p, k, pl.ds(g * 8, 8), :] = w

    def stage_u(k, n, ps):
        if all(p in RAW for p in ps):
            return
        us = pl.ds(_mo(k * 64, 64), 64)
        w0_, w1_, w2_ = [_unpack(wu[n, q, us]) for q in range(3)]
        res = [{}, {}]
        for h in range(2):
            w0, w1, w2, r = w0_[h], w1_[h], w2_[h], res[h]
            if 2 in ps:
                e = 0.5 * (w2 + w0)
                o = 0.5 * w1
                r[2] = e + o
                r[3] = e - o
            if 6 in ps:
                gr = w2 - w0
                r[6] = gr
                r[8] = gr + w1
                r[7] = w1 - gr
            if 4 in ps:
                e = MUA * (w2 + AL * w0)
                o = (MUA * A) * w1
                r[4] = e + o
                r[5] = e - o
            if 9 in ps:
                e = MUB * (AL * w2 + w0)
                o = (MUB * A) * w1
                r[9] = e + o
                r[10] = e - o
        for p in ps:
            if p not in RAW:
                u_ref[p - 2, n, us] = _pack_round(res[0][p], res[1][p])

    def rhs_ref(p, n):
        return wu.at[n, RAW[p]] if p in RAW else u_ref.at[p - 2, n]

    emitted = {}
    keep = []

    def unit_c(mview, b0, nb, first, n, g, z=None):
        keep.append(mview)
        ns = slice(n * 128, (n + 1) * 128)
        sc = p_ref[0, :, ns]
        sh = p_ref[1, :, ns]
        m0, mi, mp1, mm1, mpa, mma, q1, q2, q3, mpb, mmb = [
            mview(p, n)[pl.ds((g // 2) * 16 + (g % 2), 8, stride=2), :] for p in range(NP)]
        if z is not None:
            mp1, mpa, mpb, q1 = [_f32(_bits(a) | z) for a in (mp1, mpa, mpb, q1)]
        s1_ = mp1 + mm1
        d1_ = mp1 - mm1
        sa = mpa + mma
        da = mpa - mma
        sb = mpb + mmb
        db = mpb - mmb
        re = q1 - q3
        im = q1 + q2
        km0 = K3 * m0
        kmi = K3 * mi
        s2 = (K1 * s1_ - (sa + sb)) + km0
        s1 = (s1_ - m0) - s2
        d2 = (K4 * (sa - sb) + K6 * re) - km0
        d1 = (m0 - re) + d2
        ada = A * da
        bdb = (1.0 / A) * db
        t2 = (K1 * d1_ - (ada + bdb)) + kmi
        t1 = (d1_ - mi) - t2
        e2 = (K4 * (ada - bdb) - K6 * im) + kmi
        e1 = (im - mi) + e2
        ys = [t1 + e1, s1 + d1, t2 + e2, s2 + d2, t2 - e2, s2 - d2, t1 - e1, s1 - d1]
        outs = []
        for y in ys:
            h = y * sc + sh
            outs.append(h * jnp.tanh(h) + h)
        oc = (ou0 if first else ou).at[n, pl.ds(_mo(b0 * 4, 64), nb * 4)]
        for j in range(4):
            oc[pl.ds(g * 32 + j, 8, stride=4), :] = _pack_rne(outs[2 * j], outs[2 * j + 1])
        emitted[(id(mview), n)] = emitted.get((id(mview), n), 0) + 1
        if g == nb // 8 - 1:
            assert emitted[(id(mview), n)] == nb // 8
            o_copy(b0, nb, n, first).start()

    def c_units(c, slot):
        mv = lambda p, n: m_ref.at[slot, p, n]
        return [functools.partial(unit_c, mv, c * TB, TB, False, n, g)
                for n in range(NT) for g in range(TB // 8)]

    def cx_units(b0, nb):
        mv = lambda p, n: mp_ref.at[p, n, pl.ds(_mo(b0, 16), nb)]
        return [functools.partial(unit_c, mv, b0, nb, True, n, g)
                for n in range(NT) for g in range(nb // 8)]

    def a_units(c, ps):
        return [functools.partial(unit_a, c, k, g, ps, False) for k in range(NT) for g in range(NG)]

    def run_paced(dots, sched):
        sched = sorted(sched, key=lambda t: t[0])
        si = 0
        for d, dt in enumerate(dots):
            m = dt()
            nrow = m.shape[0] // 8
            zc = {}
            while si < len(sched) and sched[si][0] < d + 1:
                if len(sched[si]) > 2:
                    sched[si][1]()
                else:
                    i = int((sched[si][0] - d) * nrow)
                    if i not in zc:
                        zc[i] = zero_from(m, i)
                    sched[si][1](z=zc[i])
                si += 1
        assert si == len(sched)

    def mk_dot(slot, p, n, h=0, nb=TB):
        def f():
            rs = slice(h * nb // 2, (h + 1) * nb // 2)
            lhs = jnp.concatenate([pltpu.bitcast(v_ref[p, k, rs], BF16) for k in range(NT)], axis=1)
            m = jnp.dot(lhs, pltpu.bitcast(rhs_ref(p, n)[...], BF16), preferred_element_type=F32)
            m_ref[slot, p, n, h * nb:(h + 1) * nb] = m
            return m
        return f

    def gdots(ps, slot):
        return [mk_dot(slot, p, n) for n in range(NT) for p in ps]

    def p_step(k, first, jobs, a_chunks, u_ns, pace=True, pg=PG):
        def mk(p, n, cs, pre):
            def f():
                for fn in pre:
                    fn()
                h = TB // 2
                lhs = pltpu.bitcast(vp_ref[p, cs[0] * h:(cs[-1] + 1) * h], BF16)
                rhs = pltpu.bitcast(rhs_ref(p, n)[pl.ds(_mo(k * 64, 64), 64)], BF16)
                m = jnp.dot(lhs, rhs, preferred_element_type=F32)
                for i, cx in enumerate(cs):
                    dst = mp_ref.at[p, n] if cx == 0 else m_ref.at[0, p, n]
                    piece = m[i * TB:(i + 1) * TB]
                    if first:
                        dst[...] = piece
                    else:
                        dst[...] += piece
                return m
            return f
        dots, sched = [], []
        lo = PLO
        for ps in pg:
            lst = sorted([(n, ps.index(p), p, cs) for p in ps for (n, cs) in jobs(p)])
            aus = [functools.partial(unit_a, cx, k, g, ps, True) for cx in a_chunks for g in range(NG)]
            start = len(dots)
            pre = [functools.partial(stage_u, k, nn, ps) for nn in u_ns]
            if pace and len(ps) > 1 and start - PM > lo:
                sched += _spread(aus, lo, start - PM)
                lo = start - PM
            else:
                pre = aus + pre
            for i, (n, _, p, cs) in enumerate(lst):
                dots.append(mk(p, n, cs, pre if i == 0 else []))
        run_paced(dots, sched)

    both = lambda p: (0, 1) if p in G0 else (0,)

    z0_ref[...] = jnp.zeros((8, 128), U32)
    for grp in (grp_x(), grp_0a(), grp_0b(), slab(1), slab(2), slab(3), slab(4), grp_l0(), grp_l1()):
        for cp in grp:
            cp.start()

    for cp in grp_x():
        cp.wait()
    for g in range(NG):
        unit_a(0, 0, g, tuple(range(NP)), True)
    for cp in grp_0a():
        cp.wait()
    p_step(0, True, lambda p: [(n, (0,)) for n in range(N0A)], (), range(N0A), pace=False, pg=PG0A)
    for cp in grp_0b():
        cp.wait()
    mean, var, gam, bet = [q[...].astype(F32).reshape(1, C) for q in (bn0, bn1, bn2, bn3)]
    scale = gam / jnp.sqrt(var + 1e-5)
    p_ref[0] = jnp.broadcast_to(0.25 * scale, (8, C))
    p_ref[1] = jnp.broadcast_to(0.5 * (bet - mean * scale), (8, C))
    p_step(0, True,
           lambda p: ([(n, (1,)) for n in range(N0A)] if p in G0 else []) + [(n, both(p)) for n in range(N0A, NT)],
           (1,), range(N0A, NT))

    def pbody(k, carry):
        for cp in slab(k):
            cp.wait()
        p_step(k, False, lambda p: [(n, both(p)) for n in range(NT)], (0, 1), range(NT))
        return carry
    lax.fori_loop(1, NT, pbody, 0)

    def body(it, carry):
        @pl.when(it == 0)
        def _():
            for cp in grp_l0():
                cp.wait()

        @pl.when(it == 1)
        def _():
            for cp in grp_l1():
                cp.wait()
        dots, items = [], []
        xun = cx_units(it * XB, XB)
        per = len(xun) // L
        end = 55 * L - MARGIN
        for j in range(L):
            c = L * it + 1 + j
            base = 55 * j
            dots += gdots(G1, j % L) + gdots(G0, (j + 1) % L)
            endm = MARGIN if j == L - 1 else MA
            items += [(pos, base - 0.9, base + 25 - MA, COST_A, u)
                      for pos, u in _spread(a_units(c + 1, G0), base + A_LO, base + 25 - MA)]
            items += [(pos, base + 24.1, base + 55 - endm, COST_A, u)
                      for pos, u in _spread(a_units(c + 1, G1), base + A1_LO, base + 55 - endm)]
            cus = xun[j * per:(j + 1) * per] + c_units(c, j % L)
            for i, (pos, u) in enumerate(_spread(cus, base + X_LO, base + C_HI)):
                lo_ = 0.0 if i < per else base + 5 * u.args[4] + 4.5
                hi_ = min(end, base + 79.0)
                items.append((max(pos, lo_), lo_, hi_, COST_C, u))
        items.sort(key=lambda t: t[0])
        tot = sum(t[3] for t in items)
        acc = 0.0
        sched = []
        for _, lo_, hi_, cost, u in items:
            p_ = U_LO + (end - U_LO) * acc / tot
            acc += cost
            sched.append((min(max(p_, lo_, 0.0), hi_), u))
        run_paced(dots, sched)
        return carry
    lax.fori_loop(0, NIT, body, 0)

    cl = NCH - 1
    nb = TB // ESPLIT

    def blk_units(n, h):
        mv = lambda p, n_: m_ref.at[0, p, n_, pl.ds(h * nb, nb)]
        return [functools.partial(unit_c, mv, cl * TB + h * nb, nb, False, n, g) for g in range(nb // 8)]
    sched = _spread(cx_units(NIT * XB, TB - NIT * XB), EX[0], EX[1])
    ul = c_units(cl, 0)[:48] + [u for h in range(ESPLIT) for u in blk_units(NT - 2, h)]
    for n in range(NT - 1):
        span = ESPAN if n < NT - 2 else ESPAN3
        for g in range(16):
            sched.append((5 * (n + 1) + E_OFF + span * g / 16, ul[n * 16 + g]))
    for h in range(ESPLIT):
        sched += [(20 + 5 * (h + 1) - 0.5, u, True) for u in blk_units(NT - 1, h)]
    run_paced(gdots(G1, 0)[:20] + [mk_dot(0, p, NT - 1, h, nb) for h in range(ESPLIT) for p in G1], sched)

    for k in range(NT):
        for it in range(NIT):
            o_copy(it * XB, XB, k, True).wait()
        o_copy(NIT * XB, TB - NIT * XB, k, True).wait()
        for c in range(1, NCH):
            if not (c == cl and k >= NT - 2):
                o_copy(c * TB, TB, k, False).wait()
    for h in range(ESPLIT):
        for k in (NT - 2, NT - 1):
            o_copy(cl * TB + h * nb, nb, k, False).wait()


@jax.jit
def pallas_standalone__batchnorm__sampling_kernel(
    x: jax.Array,
    w: jax.Array,
    mean: jax.Array,
    var: jax.Array,
    g: jax.Array,
    b: jax.Array,
):
    assert x.shape == (B, S, C) and w.shape == (3, C, C)
    x2d = x.reshape(B * S, C)
    xtile = x.reshape(B, S, NT, 128).transpose(0, 2, 1, 3).reshape(B * NT * S, 128)
    anyspec = pl.BlockSpec(memory_space=pl.ANY)
    out = pl.pallas_call(
        _kernel,
        in_specs=[anyspec] * 7,
        out_specs=anyspec,
        out_shape=jax.ShapeDtypeStruct((B * S, C), x.dtype),
        scratch_shapes=[
            pltpu.VMEM((NT, 2 * RB, 128), BF16),
            pltpu.VMEM((B * NT * S, 128), BF16),
            pltpu.VMEM((NT, B * S, 128), BF16),
            pltpu.VMEM((NT, RB, 128), BF16),
            pltpu.VMEM((NT, 3, C, 128), BF16),
            pltpu.VMEM((NP - 2, NT, C // 2, 128), U32),
            pltpu.VMEM((C,), BF16), pltpu.VMEM((C,), BF16), pltpu.VMEM((C,), BF16), pltpu.VMEM((C,), BF16),
            pltpu.VMEM((2, 8, C), F32),
            pltpu.VMEM((8, 128), U32), pltpu.VMEM((8, 128), U32),
            pltpu.VMEM((NP, TB, 128), U32),
            pltpu.VMEM((NP, NT, TB // 2, 128), U32),
            pltpu.VMEM((NP, NT, TB, 128), F32),
            pltpu.VMEM((L, NP, NT, TB, 128), F32),
            pltpu.SemaphoreType.DMA((9,)),
            pltpu.SemaphoreType.DMA,
        ],
        compiler_params=pltpu.CompilerParams(
            vmem_limit_bytes=64 * 1024 * 1024,
            disable_bounds_checks=True,
            disable_semaphore_checks=True,
        ),
    )(x2d, xtile, w, mean, var, g, b)
    return out.reshape(B, S, C)
```

```python
import functools

import jax
import jax.numpy as jnp
from jax import lax
import jax.experimental.pallas as pl
import jax.experimental.pallas.tpu as pltpu

F32 = jnp.float32
BF16 = jnp.bfloat16
U32 = jnp.uint32

B = 1024
S = 8
C = 640
NT = C // 128
TB = 128
NCH = B // TB
RB = TB * S
G = 16
NG = TB // G
HI = 0xFFFF0000

NP = 11
G0 = (0, 1, 2, 3, 4, 5)
G1 = (6, 7, 8, 9, 10)
RAW = {0: 2, 1: 0}
A = 0.5
AL = A * A
_A1 = 1 + AL ** 3
_A2 = AL + AL ** 2
_B1 = 1 - AL ** 3
_B2 = AL - AL ** 2
_KAP = _A1 - _A2
MUA = 1 / (2 * AL * _KAP)
MUB = MUA * A
K1 = _A1 / _KAP
K3 = (1 / AL + AL ** 4) / _KAP - K1
K4 = _KAP / (_B1 + _B2)
K6 = _B1 / (_B1 + _B2)

L = 2
NIT = (NCH - 2) // L
XB = 96 // NIT
N0A = 3
PG = ((0,), (1,), (2, 3, 6, 7, 8), (4, 5), (9, 10))
PG0A = ((0,), (1,), (2, 3, 6, 7, 8), (4, 5, 9, 10))
PM, PLO = 3.6, 0.08
MA, MARGIN, A_LO, A1_LO, C_HI, X_LO, U_LO = 0.43, 1.79, 0.66, 24.9, 54.75, 0.5, 0.09
COST_A, COST_C = 140.0, 110.0
EB = (1, 1, 2, 4, 4)
EX, E_OFF, E_TAU, E_END = (0.03, 4.75), -0.5, 0.251, 0.61


def _bits(a):
    return pltpu.bitcast(a, U32)


def _f32(a):
    return pltpu.bitcast(a, F32)


def _unpack(v, dep=None):
    if dep is None:
        return _f32(v << 16), _f32(v & jnp.uint32(HI))
    sh, mask = dep
    return _f32(v << sh), _f32(v & mask)


def _pack_exact(lo, hi):
    return (_bits(lo) >> 16) | _bits(hi)


def _pack_round(lo, hi):
    half = jnp.uint32(0x8000)
    return ((_bits(lo) + half) >> 16) | ((_bits(hi) + half) & jnp.uint32(HI))


def _pack_rne(lo, hi):
    return _pack_exact(lo.astype(BF16).astype(F32), hi.astype(BF16).astype(F32))


def _mo(i, m):
    return i if isinstance(i, int) else pl.multiple_of(i, m)


def _spread(units, lo, hi):
    n = len(units)
    return [(lo + (hi - lo) * i / n, u) for i, u in enumerate(units)]


def _kernel(x_hbm, xt_hbm, w_hbm, mean_hbm, var_hbm, g_hbm, b_hbm, o_hbm,
            xbuf, xtbuf, obuf, obuf0, wbuf, u_ref, bn0, bn1, bn2, bn3, p_ref, z0_ref, z_ref,
            vp_ref, v_ref, mp_ref, m_ref, isem, osem):

    def xk_copy(k, s):
        return pltpu.make_async_copy(
            x_hbm.at[pl.ds(0, 2 * RB), pl.ds(_mo(k * 128, 128), 128)], xbuf.at[k], isem.at[s])

    def xk0_copy(c, s):
        return pltpu.make_async_copy(
            x_hbm.at[pl.ds(c * RB, RB), pl.ds(0, 128)], xbuf.at[0, pl.ds(c * RB, RB)], isem.at[s])

    def wn_copy(k, n, s):
        r0 = _mo(k * 128, 128)
        return pltpu.make_async_copy(
            w_hbm.at[:, pl.ds(r0, 128), pl.ds(n * 128, 128)], wbuf.at[n, :, pl.ds(r0, 128)], isem.at[s])

    def xt_copy(c0, nc, s):
        rows = pl.ds(c0 * TB * 40, nc * TB * 40)
        return pltpu.make_async_copy(xt_hbm.at[rows], xtbuf.at[rows], isem.at[s])

    def o_copy(b0, nb, k, first):
        r0 = _mo(b0 * S, 128)
        src = obuf0 if first else obuf
        return pltpu.make_async_copy(
            src.at[k, pl.ds(r0, nb * S)], o_hbm.at[pl.ds(r0, nb * S), pl.ds(k * 128, 128)], osem)

    def grp_x():
        return [xk0_copy(0, 8)]

    def grp_0a():
        return [wn_copy(0, n, 0) for n in range(N0A)] + [pltpu.make_async_copy(z0_ref, z_ref, isem.at[0])]

    def grp_0b():
        return ([wn_copy(0, n, 1) for n in range(N0A, NT)] + [xk0_copy(1, 1)]
                + [pltpu.make_async_copy(s_, d_, isem.at[1])
                   for s_, d_ in zip((mean_hbm, var_hbm, g_hbm, b_hbm), (bn0, bn1, bn2, bn3))])

    def slab(k):
        return [xk_copy(k, k + 1)] + [wn_copy(k, n, k + 1) for n in range(NT)]

    def grp_l0():
        return [xt_copy(2, L, 6)]

    def grp_l1():
        return [xt_copy(2 + L, NCH - 2 - L, 7)]

    def zero_from(m, i):
        return _bits(m[8 * i:8 * i + 8, 0:128]) & z_ref[...]

    def unit_a(cx, k, g, ps, pro, z=None):
        dep = None if z is None else (z | jnp.uint32(16), z | jnp.uint32(HI))
        if pro:
            xg = xbuf.at[k, pl.ds((cx * TB + g * G) * 8, G * 8)].bitcast(U32)
            off, bs = 0, 4
        else:
            xg = xtbuf.at[pl.ds(_mo((cx * TB + g * G) * 40, G * 40), G * 40)].bitcast(U32)
            off, bs = k * 4, 20
        full = any(p >= 2 for p in ps)
        vals = []
        for hf in range(2):
            x = {}
            for j in range(4):
                if full or (j == 0 and 0 in ps) or (j == 3 and 1 in ps):
                    x[2 * j], x[2 * j + 1] = _unpack(xg[pl.ds(hf * 8 * bs + off + j, 8, stride=bs), :], dep)
            v = {}
            if 0 in ps:
                v[0] = x[0]
            if 1 in ps:
                v[1] = x[7]
            if 2 in ps or 6 in ps:
                p_ = x[0] + x[4]
                q_ = x[2] + x[6]
                r_ = x[1] + x[5]
                s_ = x[3] + x[7]
            if 2 in ps:
                e1 = p_ + q_
                o1 = r_ + s_
                v[2] = e1 + o1
                v[3] = e1 - o1
            if 6 in ps:
                ei = p_ - q_
                oi = r_ - s_
                v[6] = ei + oi
                v[7] = ei
                v[8] = oi
            if 4 in ps:
                ea = x[0] + AL * (x[2] + AL * (x[4] + AL * x[6]))
                oa = A * (x[1] + AL * (x[3] + AL * (x[5] + AL * x[7])))
                v[4] = ea + oa
                v[5] = ea - oa
            if 9 in ps:
                eb = A * (x[6] + AL * (x[4] + AL * (x[2] + AL * x[0])))
                ob = x[7] + AL * (x[5] + AL * (x[3] + AL * x[1]))
                v[9] = eb + ob
                v[10] = eb - ob
            vals.append(v)
        for p in ps:
            w = (_pack_exact if p in RAW else _pack_round)(vals[0][p], vals[1][p])
            if pro and not (cx == 1 and p in G1):
                vp_ref[p, pl.ds(cx * (TB // 2) + g * 8, 8), :] = w
            else:
                v_ref[p, k, pl.ds(g * 8, 8), :] = w

    def w_tile(q, k, n):
        if k is None:
            return wbuf.at[n, q].bitcast(U32)[...]
        return wbuf.at[n, q, pl.ds(_mo(k * 128, 128), 128)].bitcast(U32)[...]

    def stage_u(k, n, ps):
        if all(p in RAW for p in ps):
            return
        us = pl.ds(_mo(k * 64, 64), 64)
        w0_, w1_, w2_ = [_unpack(w_tile(q, k, n)) for q in range(3)]
        res = [{}, {}]
        for h in range(2):
            w0, w1, w2, r = w0_[h], w1_[h], w2_[h], res[h]
            if 2 in ps:
                e = 0.5 * (w2 + w0)
                o = 0.5 * w1
                r[2] = e + o
                r[3] = e - o
            if 6 in ps:
                gr = w2 - w0
                r[6] = gr
                r[8] = gr + w1
                r[7] = w1 - gr
            if 4 in ps:
                e = MUA * (w2 + AL * w0)
                o = (MUA * A) * w1
                r[4] = e + o
                r[5] = e - o
            if 9 in ps:
                e = MUB * (AL * w2 + w0)
                o = (MUB * A) * w1
                r[9] = e + o
                r[10] = e - o
        for p in ps:
            if p not in RAW:
                u_ref[p - 2, n, us] = _pack_round(res[0][p], res[1][p])

    def rhs(p, n, k=None):
        if p in RAW:
            u = w_tile(RAW[p], k, n)
        elif k is None:
            u = u_ref[p - 2, n]
        else:
            u = u_ref[p - 2, n, pl.ds(_mo(k * 64, 64), 64)]
        return pltpu.bitcast(u, BF16)

    emitted = {}
    keep = []

    def unit_c(mview, b0, nb, first, n, g, z=None):
        keep.append(mview)
        ns = slice(n * 128, (n + 1) * 128)
        sc = p_ref[0, :, ns]
        sh = p_ref[1, :, ns]
        m0, mi, mp1, mm1, mpa, mma, q1, q2, q3, mpb, mmb = [
            mview(p, n)[pl.ds((g // 2) * 16 + (g % 2), 8, stride=2), :] for p in range(NP)]
        if z is not None:
            mp1, mpa, mpb, q1 = [_f32(_bits(a) | z) for a in (mp1, mpa, mpb, q1)]
        s1_ = mp1 + mm1
        d1_ = mp1 - mm1
        sa = mpa + mma
        da = mpa - mma
        sb = mpb + mmb
        db = mpb - mmb
        re = q1 - q3
        im = q1 + q2
        km0 = K3 * m0
        kmi = K3 * mi
        s2 = (K1 * s1_ - (sa + sb)) + km0
        s1 = (s1_ - m0) - s2
        d2 = (K4 * (sa - sb) + K6 * re) - km0
        d1 = (m0 - re) + d2
        ada = A * da
        bdb = (1.0 / A) * db
        t2 = (K1 * d1_ - (ada + bdb)) + kmi
        t1 = (d1_ - mi) - t2
        e2 = (K4 * (ada - bdb) - K6 * im) + kmi
        e1 = (im - mi) + e2
        ys = [t1 + e1, s1 + d1, t2 + e2, s2 + d2, t2 - e2, s2 - d2, t1 - e1, s1 - d1]
        outs = []
        for y in ys:
            h = y * sc + sh
            outs.append(h * jnp.tanh(h) + h)
        oc = (obuf0 if first else obuf).at[n, pl.ds(_mo((b0 + g * 8) * S, 64), 64)].bitcast(U32)
        for j in range(4):
            oc[pl.ds(j, 8, stride=4), :] = _pack_rne(outs[2 * j], outs[2 * j + 1])
        emitted[(id(mview), n)] = emitted.get((id(mview), n), 0) + 1
        if g == nb // 8 - 1:
            assert emitted[(id(mview), n)] == nb // 8
            o_copy(b0, nb, n, first).start()

    def c_units(c, slot):
        mv = lambda p, n: m_ref.at[slot, p, n]
        return [functools.partial(unit_c, mv, c * TB, TB, False, n, g)
                for n in range(NT) for g in range(TB // 8)]

    def cx_units(b0, nb):
        mv = lambda p, n: mp_ref.at[p, n, pl.ds(_mo(b0, 16), nb)]
        return [functools.partial(unit_c, mv, b0, nb, True, n, g)
                for n in range(NT) for g in range(nb // 8)]

    def a_units(c, ps):
        return [functools.partial(unit_a, c, k, g, ps, False) for k in range(NT) for g in range(NG)]

    def run_paced(dots, sched):
        sched = sorted(sched, key=lambda t: t[0])
        si = 0
        for d, dt in enumerate(dots):
            m = dt()
            nrow = m.shape[0] // 8
            zc = {}
            while si < len(sched) and sched[si][0] < d + 1:
                if len(sched[si]) > 2:
                    sched[si][1]()
                else:
                    i = int((sched[si][0] - d) * nrow)
                    if i not in zc:
                        zc[i] = zero_from(m, i)
                    sched[si][1](z=zc[i])
                si += 1
        assert si == len(sched)

    def mk_dot(slot, p, n, h=0, nb=TB):
        def f():
            rs = slice(h * nb // 2, (h + 1) * nb // 2)
            lhs = jnp.concatenate([pltpu.bitcast(v_ref[p, k, rs], BF16) for k in range(NT)], axis=1)
            m = jnp.dot(lhs, rhs(p, n), preferred_element_type=F32)
            m_ref[slot, p, n, h * nb:(h + 1) * nb] = m
            return m
        return f

    def gdots(ps, slot):
        return [mk_dot(slot, p, n) for n in range(NT) for p in ps]

    def p_step(k, first, jobs, a_chunks, u_ns, pace=True, pg=PG):
        def mk(p, n, cs, pre):
            def f():
                for fn in pre:
                    fn()
                h = TB // 2
                lhs = pltpu.bitcast(vp_ref[p, cs[0] * h:(cs[-1] + 1) * h], BF16)
                m = jnp.dot(lhs, rhs(p, n, k), preferred_element_type=F32)
                for i, cx in enumerate(cs):
                    dst = mp_ref.at[p, n] if cx == 0 else m_ref.at[0, p, n]
                    piece = m[i * TB:(i + 1) * TB]
                    if first:
                        dst[...] = piece
                    else:
                        dst[...] += piece
                return m
            return f
        dots, sched = [], []
        lo = PLO
        for ps in pg:
            lst = sorted([(n, ps.index(p), p, cs) for p in ps for (n, cs) in jobs(p)])
            aus = [functools.partial(unit_a, cx, k, g, ps, True) for cx in a_chunks for g in range(NG)]
            start = len(dots)
            pre = [functools.partial(stage_u, k, nn, ps) for nn in u_ns]
            if pace and len(ps) > 1 and start - PM > lo:
                sched += _spread(aus, lo, start - PM)
                lo = start - PM
            else:
                pre = aus + pre
            for i, (n, _, p, cs) in enumerate(lst):
                dots.append(mk(p, n, cs, pre if i == 0 else []))
        run_paced(dots, sched)

    both = lambda p: (0, 1) if p in G0 else (0,)

    z0_ref[...] = jnp.zeros((8, 128), U32)
    for grp in (grp_x(), grp_0a(), grp_0b(), slab(1), slab(2), slab(3), slab(4), grp_l0(), grp_l1()):
        for cp in grp:
            cp.start()

    for cp in grp_x():
        cp.wait()
    for g in range(NG):
        unit_a(0, 0, g, tuple(range(NP)), True)
    for cp in grp_0a():
        cp.wait()
    p_step(0, True, lambda p: [(n, (0,)) for n in range(N0A)], (), range(N0A), pace=False, pg=PG0A)
    for cp in grp_0b():
        cp.wait()
    mean, var, gam, bet = [q[...].astype(F32).reshape(1, C) for q in (bn0, bn1, bn2, bn3)]
    scale = gam / jnp.sqrt(var + 1e-5)
    p_ref[0] = jnp.broadcast_to(0.25 * scale, (8, C))
    p_ref[1] = jnp.broadcast_to(0.5 * (bet - mean * scale), (8, C))
    p_step(0, True,
           lambda p: ([(n, (1,)) for n in range(N0A)] if p in G0 else []) + [(n, both(p)) for n in range(N0A, NT)],
           (1,), range(N0A, NT))

    def pbody(k, carry):
        for cp in slab(k):
            cp.wait()
        p_step(k, False, lambda p: [(n, both(p)) for n in range(NT)], (0, 1), range(NT))
        return carry
    lax.fori_loop(1, NT, pbody, 0)

    def body(it, carry):
        @pl.when(it == 0)
        def _():
            for cp in grp_l0():
                cp.wait()

        @pl.when(it == 1)
        def _():
            for cp in grp_l1():
                cp.wait()
        dots, items = [], []
        xun = cx_units(it * XB, XB)
        per = len(xun) // L
        end = 55 * L - MARGIN
        for j in range(L):
            c = L * it + 1 + j
            base = 55 * j
            dots += gdots(G1, j % L) + gdots(G0, (j + 1) % L)
            endm = MARGIN if j == L - 1 else MA
            items += [(pos, base - 0.9, base + 25 - MA, COST_A, u)
                      for pos, u in _spread(a_units(c + 1, G0), base + A_LO, base + 25 - MA)]
            items += [(pos, base + 24.1, base + 55 - endm, COST_A, u)
                      for pos, u in _spread(a_units(c + 1, G1), base + A1_LO, base + 55 - endm)]
            cus = xun[j * per:(j + 1) * per] + c_units(c, j % L)
            for i, (pos, u) in enumerate(_spread(cus, base + X_LO, base + C_HI)):
                lo_ = 0.0 if i < per else base + 5 * u.args[4] + 4.5
                hi_ = min(end, base + 79.0)
                items.append((max(pos, lo_), lo_, hi_, COST_C, u))
        items.sort(key=lambda t: t[0])
        tot = sum(t[3] for t in items)
        acc = 0.0
        sched = []
        for _, lo_, hi_, cost, u in items:
            p_ = U_LO + (end - U_LO) * acc / tot
            acc += cost
            sched.append((min(max(p_, lo_, 0.0), hi_), u))
        run_paced(dots, sched)
        return carry
    lax.fori_loop(0, NIT, body, 0)

    cl = NCH - 1
    blocks = [(n, h, TB // sp) for n, sp in enumerate(EB) for h in range(sp)]
    dots, t_start = [], [0.0]
    for (n, h, nb) in blocks:
        for p in G1:
            dots.append(mk_dot(0, p, n, h, nb))
            t_start.append(t_start[-1] + nb / TB)

    def pos_of(t):
        for d in range(len(dots)):
            if t < t_start[d + 1]:
                return d + (t - t_start[d]) / (t_start[d + 1] - t_start[d])
        return None
    sched = _spread(cx_units(NIT * XB, TB - NIT * XB), EX[0], EX[1])
    t = 0.0
    for i, (n, h, nb) in enumerate(blocks):
        mv = lambda p, n_, h=h, nb=nb: m_ref.at[0, p, n_, pl.ds(h * nb, nb)]
        last = 5 * i + 4
        t = max(t, t_start[last + 1] + E_OFF * nb / TB)
        for g in range(nb // 8):
            u = functools.partial(unit_c, mv, cl * TB + h * nb, nb, False, n, g)
            pos = pos_of(t)
            if pos is None or t > t_start[-1] - E_END:
                prev = sched[-1][0]
                sched.append((max(last + 0.5, prev), u, True))
            else:
                sched.append((max(pos, last + 0.01), u))
            t += E_TAU
    run_paced(dots, sched)

    for k in range(NT):
        for it in range(NIT):
            o_copy(it * XB, XB, k, True).wait()
        o_copy(NIT * XB, TB - NIT * XB, k, True).wait()
        for c in range(1, NCH - 1):
            o_copy(c * TB, TB, k, False).wait()
    for (n, h, nb) in blocks:
        o_copy(cl * TB + h * nb, nb, n, False).wait()


@jax.jit
def pallas_standalone__batchnorm__sampling_kernel(
    x: jax.Array,
    w: jax.Array,
    mean: jax.Array,
    var: jax.Array,
    g: jax.Array,
    b: jax.Array,
):
    assert x.shape == (B, S, C) and w.shape == (3, C, C)
    x2d = x.reshape(B * S, C)
    xtile = x.reshape(B, S, NT, 128).transpose(0, 2, 1, 3).reshape(B * NT * S, 128)
    anyspec = pl.BlockSpec(memory_space=pl.ANY)
    out = pl.pallas_call(
        _kernel,
        in_specs=[anyspec] * 7,
        out_specs=anyspec,
        out_shape=jax.ShapeDtypeStruct((B * S, C), x.dtype),
        scratch_shapes=[
            pltpu.VMEM((NT, 2 * RB, 128), BF16),
            pltpu.VMEM((B * NT * S, 128), BF16),
            pltpu.VMEM((NT, B * S, 128), BF16),
            pltpu.VMEM((NT, RB, 128), BF16),
            pltpu.VMEM((NT, 3, C, 128), BF16),
            pltpu.VMEM((NP - 2, NT, C // 2, 128), U32),
            pltpu.VMEM((C,), BF16), pltpu.VMEM((C,), BF16), pltpu.VMEM((C,), BF16), pltpu.VMEM((C,), BF16),
            pltpu.VMEM((2, 8, C), F32),
            pltpu.VMEM((8, 128), U32), pltpu.VMEM((8, 128), U32),
            pltpu.VMEM((NP, TB, 128), U32),
            pltpu.VMEM((NP, NT, TB // 2, 128), U32),
            pltpu.VMEM((NP, NT, TB, 128), F32),
            pltpu.VMEM((L, NP, NT, TB, 128), F32),
            pltpu.SemaphoreType.DMA((9,)),
            pltpu.SemaphoreType.DMA,
        ],
        compiler_params=pltpu.CompilerParams(
            vmem_limit_bytes=64 * 1024 * 1024,
            disable_bounds_checks=True,
            disable_semaphore_checks=True,
        ),
    )(x2d, xtile, w, mean, var, g, b)
    return out.reshape(B, S, C)
```
